```python
import os as _os
_os.environ.setdefault("JAX_PLATFORMS", "cpu")
import jax
import jax.numpy as jnp

def _softmax(x, axis=-1):
    return jax.nn.softmax(x, axis=axis)
def _gelu(x):
    return jax.nn.gelu(x, approximate=True)
def _silu(x):
    return jax.nn.silu(x)
def _sigmoid(x):
    return jax.nn.sigmoid(x)
def _layernorm(x, axis=-1, eps=1e-5):
    m = jnp.mean(x, axis=axis, keepdims=True)
    v = jnp.var(x, axis=axis, keepdims=True)
    return (x - m) / jnp.sqrt(v + eps)
def _scatter_add(tgt, idx, src, axis=0):
    return tgt.at[idx].add(src)
def _segment_sum(src, seg, n):
    return jax.ops.segment_sum(src, seg, n)
class _Rng:
    def __init__(self, key):
        self._k = key
    def _next(self):
        self._k, sub = jax.random.split(self._k)
        return sub
    def normal(self, shape):
        return jax.random.normal(self._next(), shape, dtype=jnp.bfloat16)
    def randint(self, lo, hi, shape):
        return jax.random.randint(self._next(), shape, lo, hi, dtype=jnp.int32)
    def uniform(self, shape, lo=0.0, hi=1.0):
        return jax.random.uniform(self._next(), shape, jnp.bfloat16, lo, hi)
    def permutation(self, n):
        return jax.random.permutation(self._next(), n)


kernel_name = 'concat_heads__softmax_full_mha__ssm_conv_s5__prompt'

def setup_inputs():
    _rng = _Rng(jax.random.key(int.from_bytes(__import__("os").urandom(4), "little")))
    _w = (lambda a: (lambda t: t.astype(jnp.bfloat16) if jnp.issubdtype(t.dtype, jnp.floating) else t)(jnp.asarray(a)))
    def _A_setup():
        B, S, D = 1, 2048, 512
        return {
            "x": _w((lambda *s: _rng.normal(s) * 0.2)(B, S, D)),
            "wqkv": _w((lambda *s: _rng.normal(s) * 0.2)(D, 3 * D)),
            "wo": _w((lambda *s: _rng.normal(s) * 0.05)(D, D)),
        }
    _A_in = _A_setup()

    def _B_setup():
        B, S, D = 1, 2048, 512
        P = D
        Lambda_re = -0.5 * jnp.exp((lambda *s: _rng.normal(s) * 0.4)(P))
        Lambda_im = (lambda *s: _rng.normal(s) * 0.4)(P) * 1.0
        B_re = (lambda *s: _rng.normal(s) * 0.4)(P, D) * (D ** -0.5)
        B_im = (lambda *s: _rng.normal(s) * 0.4)(P, D) * (D ** -0.5)
        C_re = (lambda *s: _rng.normal(s) * 0.4)(D, P) * (P ** -0.5)
        C_im = (lambda *s: _rng.normal(s) * 0.4)(D, P) * (P ** -0.5)
        log_dt = (lambda *s: _rng.normal(s) * 0.4)(P) * 0.3 - 2.0
        Dskip = (lambda *s: _rng.normal(s) * 0.4)(D)
        return {
            "x": _w((lambda *s: _rng.normal(s) * 0.05)(B, S, D)),
            "Lambda_re": _w(Lambda_re),
            "Lambda_im": _w(Lambda_im),
            "B_re": _w(B_re),
            "B_im": _w(B_im),
            "C_re": _w(C_re),
            "C_im": _w(C_im),
            "log_dt": _w(log_dt),
            "Dskip": _w(Dskip),
        }
    _B_in = _B_setup()

    return {
        "A_x": _A_in["x"],
        "A_wqkv": _A_in["wqkv"],
        "A_wo": _A_in["wo"],
        "B_x": _B_in["x"],
        "B_Lambda_re": _B_in["Lambda_re"],
        "B_Lambda_im": _B_in["Lambda_im"],
        "B_B_re": _B_in["B_re"],
        "B_B_im": _B_in["B_im"],
        "B_C_re": _B_in["C_re"],
        "B_C_im": _B_in["C_im"],
        "B_log_dt": _B_in["log_dt"],
        "B_Dskip": _B_in["Dskip"],
    }

def reference(A_x, A_wqkv, A_wo, B_x, B_Lambda_re, B_Lambda_im, B_B_re, B_B_im, B_C_re, B_C_im, B_log_dt, B_Dskip):
    def _A_ref(x, wqkv, wo):
        B, S, D = x.shape
        H = 32; Dh = D // H
        qkv = (lambda x, *d: x.transpose(*d))((x @ wqkv).reshape(B, S, 3, H, Dh), 2, 0, 3, 1, 4)
        q, k, v = qkv[0], qkv[1], qkv[2]
        scale = Dh ** -0.5
        scores = jnp.einsum("bhqd,bhkd->bhqk", q, k) * scale
        p = _softmax(scores, axis=-1)
        o = jnp.einsum("bhqk,bhkd->bhqd", p, v)
        return (lambda x, *d: x.transpose(*d))(o, 0, 2, 1, 3).reshape(B, S, D) @ wo

    def _B_ref(x, Lambda_re, Lambda_im, B_re, B_im, C_re, C_im, log_dt, Dskip):
        Bsz, L, H = x.shape
        Lam = Lambda_re + 1j * Lambda_im
        Bmat = B_re + 1j * B_im
        Cmat = C_re + 1j * C_im
        dt = jnp.exp(log_dt)
        Lam_bar = jnp.exp(dt * Lam)
        B_bar = ((Lam_bar - 1.0) / Lam)[:, None] * Bmat
        Bu = jnp.einsum("bld,pd->blp", x + 0j, B_bar)
        h = jnp.zeros_like(Bu[:, 0, :])
        hs = []
        for t in range(L):
            h = Lam_bar[None, :] * h + Bu[:, t, :]
            hs.append(h)
        hseq = jnp.stack(hs, 1)
        y = 2.0 * jnp.einsum("blp,dp->bld", hseq, Cmat).real + x * Dskip[None, None, :]
        return y

    a = _A_ref(A_x, A_wqkv, A_wo)
    b = _B_ref(B_x, B_Lambda_re, B_Lambda_im, B_B_re, B_B_im, B_C_re, B_C_im, B_log_dt, B_Dskip)
    return jnp.concatenate([a, b], axis=-1)
```

```python
import functools
import math

import jax
import jax.numpy as jnp
import jax.experimental.pallas as pl
import jax.experimental.pallas.tpu as pltpu

F32 = jnp.float32
BF16 = jnp.bfloat16

S = 2048
D = 512
H = 32
DH = 16
TQ = 512
NQB = S // TQ
HG = 8
NG = H // HG
CK = 128
DEPTH = 2
TS = TQ // NG
LOG2E = math.log2(math.e)
QSCALE = (DH ** -0.5) * LOG2E

_NN = (((1,), (0,)), ((), ()))
_NT = (((1,), (1,)), ((), ()))
_TN = (((0,), (0,)), ((), ()))


def _dot(a, b, dims=_NN):
    return jax.lax.dot_general(a, b, dims, preferred_element_type=F32)


def _cmul(ar, ai, br, bi):
    return ar * br - ai * bi, ar * bi + ai * br


def _kernel(x_ref, wqkv_ref, wo_ref, bx_ref, lre_ref, lim_ref, bre_ref, bim_ref,
            cre_ref, cim_ref, ldt_ref, dsk_ref,
            out_ref,
            qt_ref, k_ref, vt_ref, ot_ref, c1_ref, c2_ref, tab_ref, carry_ref, safe_ref):
    step = pl.program_id(0)

    @pl.when(step == 0)
    def _setup():
        lre = lre_ref[...].astype(F32).reshape(1, D)
        lim = lim_ref[...].astype(F32).reshape(1, D)
        dt = jnp.exp(ldt_ref[...].astype(F32).reshape(1, D)).astype(BF16).astype(F32)
        mag = jnp.exp(dt * lre)
        ang = dt * lim
        a1r = mag * jnp.cos(ang)
        a1i = mag * jnp.sin(ang)
        nr = a1r - 1.0
        ni = a1i
        big = jnp.abs(lre) >= jnp.abs(lim)
        u = jnp.where(big, lre, lim)
        v = jnp.where(big, lim, lre)
        r = v / u
        den = u + v * r
        cr = jnp.where(big, nr + ni * r, nr * r + ni) / den
        ci = jnp.where(big, ni - nr * r, ni * r - nr) / den
        cre = cre_ref[...].astype(F32)
        cim = cim_ref[...].astype(F32)
        c1_ref[...] = (2.0 * (cre * cr - cim * ci)).astype(BF16)
        c2_ref[...] = (-2.0 * (cre * ci + cim * cr)).astype(BF16)
        pw = [(a1r, a1i)]
        for _ in range(7):
            pw.append(_cmul(pw[-1][0], pw[-1][1], a1r, a1i))
        row = jax.lax.broadcasted_iota(jnp.int32, (8, D), 0)
        apr = jnp.zeros((8, D), F32)
        api = jnp.zeros((8, D), F32)
        for j in range(8):
            apr = jnp.where(row == j, pw[j][0], apr)
            api = jnp.where(row == j, pw[j][1], api)
        tab_ref[0] = apr
        tab_ref[1] = api
        for n, d in enumerate((1, 2, 4)):
            tab_ref[2 + 2 * n] = jnp.where(row >= d, pw[d - 1][0], 0.0)
            tab_ref[3 + 2 * n] = jnp.where(row >= d, pw[d - 1][1], 0.0)
        carry_ref[...] = jnp.zeros_like(carry_ref)

        wq_t = wqkv_ref[:, 0:D].T
        wv_t = wqkv_ref[:, 2 * D:3 * D].T
        wk = wqkv_ref[:, D:2 * D]
        qmax = jnp.zeros((H, 128), F32)
        kmax = jnp.zeros((8, D), F32)
        vmax = jnp.zeros((8, 128), F32)
        for c in range(S // TQ):
            xc = x_ref[c * TQ:(c + 1) * TQ, :]
            kc = _dot(xc, wk).astype(BF16)
            for g in range(NG):
                k_ref[g, c * TQ:(c + 1) * TQ, :] = kc[:, g * 128:(g + 1) * 128]
            kmax = jnp.maximum(kmax, jnp.abs(kc.astype(F32)).reshape(TQ // 8, 8, D).max(axis=0))
            qc = (_dot(wq_t, xc, _NT) * QSCALE).astype(BF16)
            qt_ref[:, c * TQ:(c + 1) * TQ] = qc
            qf = qc.astype(F32)
            qn = (qf * qf).reshape(H, DH, TQ).sum(axis=1)
            for t in range(TQ // 128):
                qmax = jnp.maximum(qmax, qn[:, t * 128:(t + 1) * 128])
            vc = _dot(wv_t, xc, _NT).astype(BF16)
            vt_ref[:, c * TQ:(c + 1) * TQ] = vc
            va = jnp.abs(vc.astype(F32)).reshape(D // 8, 8, TQ).max(axis=0)
            for t in range(TQ // 128):
                vmax = jnp.maximum(vmax, va[:, t * 128:(t + 1) * 128])
        kcol = kmax.max(axis=0, keepdims=True)
        kcol2 = jnp.broadcast_to(kcol * kcol, (8, D))
        ind = (jax.lax.broadcasted_iota(jnp.int32, (D, 128), 0) // DH
               == jax.lax.broadcasted_iota(jnp.int32, (D, 128), 1)).astype(F32)
        kn2 = jax.lax.dot_general(kcol2, ind, _NN, preferred_element_type=F32,
                                  precision=jax.lax.Precision.HIGHEST)
        bound = jnp.sqrt(jnp.max(qmax) * jnp.max(kn2)) * 1.02 + 1.0
        lv = jnp.log2(jnp.max(vmax))
        ok = jnp.logical_and(bound <= 80.0,
                             jnp.logical_and(lv >= bound - 100.0, lv <= 113.0 - bound))
        safe_ref[0] = ok.astype(jnp.int32)

    def ssm_chunk(g):
        r0 = pl.multiple_of(g * TS, TS)
        xb = bx_ref[pl.ds(r0, TS), :]
        ur = _dot(xb, bre_ref[...], _NT).reshape(TS // 8, 8, D)
        ui = _dot(xb, bim_ref[...], _NT).reshape(TS // 8, 8, D)
        for n, d in enumerate((1, 2, 4)):
            mr = tab_ref[2 + 2 * n]
            mi = tab_ref[3 + 2 * n]
            sr = pltpu.roll(ur, d, 1)
            si = pltpu.roll(ui, d, 1)
            ur, ui = ur + (mr * sr - mi * si), ui + (mr * si + mi * sr)
        apr = tab_ref[0]
        api = tab_ref[1]
        cr = carry_ref[0]
        ci = carry_ref[1]
        hr, hi = [], []
        for j in range(TS // 8):
            gr = ur[j] + (apr * cr - api * ci)
            gi = ui[j] + (apr * ci + api * cr)
            hr.append(gr)
            hi.append(gi)
            cr = jnp.broadcast_to(gr[7:8, :], (8, D))
            ci = jnp.broadcast_to(gi[7:8, :], (8, D))
        carry_ref[0] = cr
        carry_ref[1] = ci
        gr = jnp.concatenate(hr, axis=0).astype(BF16)
        gi = jnp.concatenate(hi, axis=0).astype(BF16)
        skip = (xb.astype(F32) * dsk_ref[...].astype(F32).reshape(1, D)).astype(BF16).astype(F32)
        y = _dot(gr, c1_ref[...], _NT) + _dot(gi, c2_ref[...], _NT) + skip
        out_ref[pl.ds(r0, TS), D:2 * D] = y

    q0 = pl.multiple_of(step * TQ, TQ)

    def masked_q(g, hh):
        qg = qt_ref[pl.ds(pl.multiple_of(g * 128, 128), 128), pl.ds(q0, TQ)]
        rows = jax.lax.broadcasted_iota(jnp.int32, (128, TQ), 0)
        return jnp.where((rows // DH) == hh, qg, jnp.zeros_like(qg))

    def group_fast(g, carry):
        nck = S // CK
        steps = [(j, kc) for j in range(HG) for kc in range(nck)]
        ws = {}

        def qk(st):
            j, kc = st
            if j not in ws:
                ws[j] = masked_q(g, j)
            return _dot(k_ref[g, kc * CK:(kc + 1) * CK, :], ws[j])

        svals = {}
        for i in range(DEPTH):
            svals[i] = qk(steps[i])
        ssm_chunk(g)
        l = o = None
        for i, (j, kc) in enumerate(steps):
            if i + DEPTH < len(steps):
                svals[i + DEPTH] = qk(steps[i + DEPTH])
            p = jnp.exp2(svals.pop(i))
            hrow = pl.multiple_of(g * 128 + j * DH, DH)
            ps = p.reshape(CK // 8, 8, TQ).sum(axis=0)
            pv = _dot(vt_ref[pl.ds(hrow, DH), kc * CK:(kc + 1) * CK], p.astype(BF16))
            if kc == 0:
                l, o = ps, pv
            else:
                l, o = l + ps, o + pv
            if kc == nck - 1:
                ot_ref[pl.ds(hrow, DH), :] = (o / l.sum(axis=0, keepdims=True)).astype(BF16)
        return carry

    def group_safe(g, carry):
        ssm_chunk(g)
        ck = 512

        def head(j, c):
            w = masked_q(g, j)
            hrow = pl.multiple_of(g * 128 + j * DH, DH)
            m = jnp.full((1, TQ), -jnp.inf, F32)
            l = jnp.zeros((1, TQ), F32)
            o = jnp.zeros((DH, TQ), F32)
            for kc in range(S // ck):
                s = _dot(k_ref[g, kc * ck:(kc + 1) * ck, :], w)
                mn = jnp.maximum(m, s.max(axis=0, keepdims=True))
                alpha = jnp.exp2(m - mn)
                p = jnp.exp2(s - mn)
                l = l * alpha + p.sum(axis=0, keepdims=True)
                o = o * alpha + _dot(vt_ref[pl.ds(hrow, DH), kc * ck:(kc + 1) * ck], p.astype(BF16))
                m = mn
            ot_ref[pl.ds(hrow, DH), :] = (o / l).astype(BF16)
            return c

        jax.lax.fori_loop(0, HG, head, 0)
        return carry

    @pl.when(safe_ref[0] == 1)
    def _():
        jax.lax.fori_loop(0, NG, group_fast, 0)

    @pl.when(safe_ref[0] != 1)
    def _():
        jax.lax.fori_loop(0, NG, group_safe, 0)

    out_ref[:, 0:D] = _dot(ot_ref[...], wo_ref[...], _TN)


@jax.jit
def pallas_concat_heads__softmax_full_mha__ssm_conv_s5__prompt_kernel(
    A_x: jax.Array,
    A_wqkv: jax.Array,
    A_wo: jax.Array,
    B_x: jax.Array,
    B_Lambda_re: jax.Array,
    B_Lambda_im: jax.Array,
    B_B_re: jax.Array,
    B_B_im: jax.Array,
    B_C_re: jax.Array,
    B_C_im: jax.Array,
    B_log_dt: jax.Array,
    B_Dskip: jax.Array,
):
    full2 = lambda shape: pl.BlockSpec(shape, lambda i: (0, 0))
    vec = pl.BlockSpec((D,), lambda i: (0,))
    out = pl.pallas_call(
        _kernel,
        grid=(NQB,),
        in_specs=[
            full2((S, D)),
            full2((D, 3 * D)),
            full2((D, D)),
            pl.BlockSpec((TQ, D), lambda i: (i, 0)),
            vec, vec,
            full2((D, D)), full2((D, D)),
            full2((D, D)), full2((D, D)),
            vec, vec,
        ],
        out_specs=pl.BlockSpec((TQ, 2 * D), lambda i: (i, 0)),
        out_shape=jax.ShapeDtypeStruct((S, 2 * D), F32),
        scratch_shapes=[
            pltpu.VMEM((D, S), BF16),
            pltpu.VMEM((NG, S, 128), BF16),
            pltpu.VMEM((D, S), BF16),
            pltpu.VMEM((D, TQ), BF16),
            pltpu.VMEM((D, D), BF16),
            pltpu.VMEM((D, D), BF16),
            pltpu.VMEM((8, 8, D), F32),
            pltpu.VMEM((2, 8, D), F32),
            pltpu.SMEM((1,), jnp.int32),
        ],
        compiler_params=pltpu.CompilerParams(
            dimension_semantics=("arbitrary",),
            vmem_limit_bytes=100 * 1024 * 1024,
        ),
    )(A_x.reshape(S, D), A_wqkv, A_wo, B_x.reshape(S, D), B_Lambda_re, B_Lambda_im,
      B_B_re, B_B_im, B_C_re, B_C_im, B_log_dt, B_Dskip)
    return out.reshape(1, S, 2 * D)
```

```python
import math

import jax
import jax.numpy as jnp
import jax.experimental.pallas as pl
import jax.experimental.pallas.tpu as pltpu

F32 = jnp.float32
BF16 = jnp.bfloat16

S = 2048
D = 512
H = 32
DH = 16
TQ = 512
NQB = S // TQ
HG = 8
NG = H // HG
CK = 128
NV = 16
NCK = S // CK
DEPTH = 2
TS = 128
TB = S // NG
SCAN_CHAINS = 2
LOG2E = math.log2(math.e)
QSCALE = (DH ** -0.5) * LOG2E

_NN = (((1,), (0,)), ((), ()))
_NT = (((1,), (1,)), ((), ()))
_TN = (((0,), (0,)), ((), ()))

(_S_WK, _S_X0, _S_WQ, _S_WV, _S_X1, _S_X2, _S_X3, _S_LRE, _S_LIM, _S_LDT, _S_DSK,
 _S_BRE, _S_BIM, _S_BX0, _S_CRE, _S_CIM, _S_BX1, _S_WO) = range(18)
_N_IN_SEMS = 18


def _dot(a, b, dims=_NN):
    return jax.lax.dot_general(a, b, dims, preferred_element_type=F32)


def _cmul(ar, ai, br, bi):
    return ar * br - ai * bi, ar * bi + ai * br


def _kernel(x_hbm, wqkv_hbm, wo_hbm, bx_hbm, lre_hbm, lim_hbm, bre_hbm, bim_hbm,
            cre_hbm, cim_hbm, ldt_hbm, dsk_hbm,
            out_hbm,
            x_ref, w_ref, wo_ref, bx_ref, bre_ref, bim_ref, cre_ref, cim_ref,
            qt_ref, k_ref, vt_ref, ot_ref, lt_ref, tab_ref, carry_ref, qf_ref, kv_ref, kb_ref,
            oacc_ref, ys_ref, lre_ref, lim_ref, ldt_ref, dsk_ref,
            safe_ref, in_sems, ys_sems, oa_sems):

    def cp(src, dst, s):
        return pltpu.make_async_copy(src, dst, in_sems.at[s])

    copies = {
        _S_WK: cp(wqkv_hbm.at[:, D:2 * D], w_ref.at[1], _S_WK),
        _S_X0: cp(x_hbm.at[0:TQ], x_ref.at[0:TQ], _S_X0),
        _S_WQ: cp(wqkv_hbm.at[:, 0:D], w_ref.at[0], _S_WQ),
        _S_WV: cp(wqkv_hbm.at[:, 2 * D:3 * D], w_ref.at[2], _S_WV),
        _S_X1: cp(x_hbm.at[TQ:2 * TQ], x_ref.at[TQ:2 * TQ], _S_X1),
        _S_X2: cp(x_hbm.at[2 * TQ:3 * TQ], x_ref.at[2 * TQ:3 * TQ], _S_X2),
        _S_X3: cp(x_hbm.at[3 * TQ:4 * TQ], x_ref.at[3 * TQ:4 * TQ], _S_X3),
        _S_LRE: cp(lre_hbm, lre_ref, _S_LRE),
        _S_LIM: cp(lim_hbm, lim_ref, _S_LIM),
        _S_LDT: cp(ldt_hbm, ldt_ref, _S_LDT),
        _S_DSK: cp(dsk_hbm, dsk_ref, _S_DSK),
        _S_BRE: cp(bre_hbm, bre_ref, _S_BRE),
        _S_BIM: cp(bim_hbm, bim_ref, _S_BIM),
        _S_BX0: cp(bx_hbm.at[0:TB], bx_ref.at[0:TB], _S_BX0),
        _S_CRE: cp(cre_hbm, cre_ref, _S_CRE),
        _S_CIM: cp(cim_hbm, cim_ref, _S_CIM),
        _S_BX1: cp(bx_hbm.at[TB:S], bx_ref.at[TB:S], _S_BX1),
        _S_WO: cp(wo_hbm, wo_ref, _S_WO),
    }
    for c in copies.values():
        c.start()

    def wait(*ids):
        for s_ in ids:
            copies[s_].wait()

    def ys_copy(g):
        r0 = pl.multiple_of(g * TB, TB)
        return pltpu.make_async_copy(ys_ref.at[pl.ds(r0, TB)],
                                     out_hbm.at[pl.ds(r0, TB), D:2 * D], ys_sems.at[g])

    def oa_copy(qb):
        r0 = pl.multiple_of(qb * TQ, TQ)
        return pltpu.make_async_copy(oacc_ref.at[pl.ds(r0, TQ)],
                                     out_hbm.at[pl.ds(r0, TQ), 0:D], oa_sems.at[qb])

    def gen_kb(g, lanes):
        blk = pltpu.bitcast(kv_ref[g], jnp.uint32)
        for c in lanes:
            col = jnp.broadcast_to(blk[:, c:c + 1], blk.shape)
            col = pltpu.bitcast(col, BF16).astype(F32)
            kb_ref[c // DH, :, c % DH] = col.reshape(NCK, NV, 128)

    def ssm_b(u):
        r0 = pl.multiple_of(u * TS, TS)
        xb = bx_ref[pl.ds(r0, TS), :]
        ur = _dot(xb, bre_ref[...], _NT).reshape(TS // 8, 8, D)
        ui = _dot(xb, bim_ref[...], _NT).reshape(TS // 8, 8, D)
        return ur, ui

    def ssm_scan(ur, ui, link):
        nl = D // 128
        ta, tb = tab_ref[0, :, 0:128], tab_ref[1, :, 0:128]
        never = jnp.logical_and(ta < tb, tb < ta)
        cs = [(carry_ref[0, :, lt * 128:(lt + 1) * 128], carry_ref[1, :, lt * 128:(lt + 1) * 128])
              for lt in range(nl)]
        hr = [[None] * nl for _ in range(TS // 8)]
        hi = [[None] * nl for _ in range(TS // 8)]
        for j in range(TS // 8):
            for lt in range(nl):
                sl = slice(lt * 128, (lt + 1) * 128)
                ch = lt * SCAN_CHAINS // nl
                xr = ur[j][:, sl]
                xi = ui[j][:, sl]
                if link[ch] is not None:
                    xr = jnp.where(never, link[ch], xr)
                for n, d in enumerate((1, 2, 4)):
                    mr = tab_ref[2 + 2 * n, :, sl]
                    mi = tab_ref[3 + 2 * n, :, sl]
                    sr = pltpu.roll(xr, d, 0)
                    si = pltpu.roll(xi, d, 0)
                    xr, xi = xr + (mr * sr - mi * si), xi + (mr * si + mi * sr)
                apr = tab_ref[0, :, sl]
                api = tab_ref[1, :, sl]
                cr, ci = cs[lt]
                gr = xr + (apr * cr - api * ci)
                gi = xi + (apr * ci + api * cr)
                c2r = tab_ref[8, :, sl]
                c2i = tab_ref[9, :, sl]
                hr[j][lt] = c2r * gr - c2i * gi
                hi[j][lt] = -(c2r * gi + c2i * gr)
                cs[lt] = (jnp.broadcast_to(gr[7:8, :], (8, 128)), jnp.broadcast_to(gi[7:8, :], (8, 128)))
                link[ch] = gr
        for lt in range(nl):
            carry_ref[0, :, lt * 128:(lt + 1) * 128] = cs[lt][0]
            carry_ref[1, :, lt * 128:(lt + 1) * 128] = cs[lt][1]
        cat = lambda h: jnp.concatenate([jnp.concatenate(r, axis=1) for r in h], axis=0).astype(BF16)
        return cat(hr), cat(hi)

    def ssm_out(u, hr, hi):
        r0 = pl.multiple_of(u * TS, TS)
        xb = bx_ref[pl.ds(r0, TS), :]
        skip = (xb.astype(F32) * dsk_ref[...].astype(F32).reshape(1, D)).astype(BF16).astype(F32)
        ys_ref[pl.ds(r0, TS), :] = (_dot(hr, cre_ref[...], _NT) + _dot(hi, cim_ref[...], _NT) + skip)

    def out_proj(g, qb):
        q0 = pl.multiple_of(qb * TQ, TQ)
        w0 = pl.multiple_of(g * 128, 128)
        den = lt_ref[qb].reshape(HG, 8, TQ).sum(axis=1, keepdims=True)
        on = (ot_ref[qb].reshape(HG, DH, TQ) / den).astype(BF16).reshape(128, TQ)
        contrib = _dot(on, wo_ref[pl.ds(w0, 128), :], _TN)
        old = jnp.where(g == 0, 0.0, oacc_ref[pl.ds(q0, TQ), :])
        oacc_ref[pl.ds(q0, TQ), :] = old + contrib

    def prep_group(g, extra):
        n = TB // TS
        u0 = g * n
        per = 128 // n
        us = [ssm_b(u0 + u) for u in range(n)]
        for u in range(n):
            extra[u]()
        link = [None] * SCAN_CHAINS
        hs = []
        for u in range(n):
            gen_kb(g, range(u * per, (u + 1) * per))
            hs.append(ssm_scan(*us[u], link))
        for u in range(n):
            ssm_out(u0 + u, *hs[u])

    stats = {"q": jnp.zeros((H, 128), F32), "k": jnp.zeros((8, D), F32), "v": jnp.zeros((8, 128), F32)}

    def k_proj(c):
        kc = _dot(x_ref[c * TQ:(c + 1) * TQ, :], w_ref[1]).astype(BF16)
        for g in range(NG):
            k_ref[g, c * TQ:(c + 1) * TQ, :] = kc[:, g * 128:(g + 1) * 128]
            for u in range(TQ // CK):
                r0 = (c * (TQ // CK) + u) * NV
                kv_ref[g, r0:r0 + NV, :] = kc[u * CK:u * CK + NV, g * 128:(g + 1) * 128]
        stats["k"] = jnp.maximum(stats["k"], jnp.abs(kc.astype(F32)).reshape(TQ // 8, 8, D).max(axis=0))

    def q_proj(c, wq_t):
        qc = (_dot(wq_t, x_ref[c * TQ:(c + 1) * TQ, :], _NT) * QSCALE).astype(BF16)
        qt_ref[:, c * TQ:(c + 1) * TQ] = qc
        qf = qc.astype(F32).reshape(H, DH, TQ)
        qf_ref[c] = qf
        qn = (qf * qf).sum(axis=1)
        for t in range(TQ // 128):
            stats["q"] = jnp.maximum(stats["q"], qn[:, t * 128:(t + 1) * 128])

    def v_proj(c, wv_t):
        vc = _dot(wv_t, x_ref[c * TQ:(c + 1) * TQ, :], _NT).astype(BF16)
        vt_ref[:, c * TQ:(c + 1) * TQ] = vc
        va = jnp.abs(vc.astype(F32)).reshape(D // 8, 8, TQ).max(axis=0)
        for t in range(TQ // 128):
            stats["v"] = jnp.maximum(stats["v"], va[:, t * 128:(t + 1) * 128])

    wait(_S_WK, _S_X0)
    k_proj(0)
    wait(_S_WQ, _S_WV)
    wq_t = w_ref[0].T
    wv_t = w_ref[2].T
    q_proj(0, wq_t)
    v_proj(0, wv_t)
    wait(_S_X1, _S_X2, _S_X3, _S_LRE, _S_LIM, _S_LDT, _S_DSK)
    for c in range(1, S // TQ):
        k_proj(c)

    lre = lre_ref[...].astype(F32).reshape(1, D)
    lim = lim_ref[...].astype(F32).reshape(1, D)
    dt = jnp.exp(ldt_ref[...].astype(F32).reshape(1, D)).astype(BF16).astype(F32)
    mag = jnp.exp(dt * lre)
    ang = dt * lim
    a1r = mag * jnp.cos(ang)
    a1i = mag * jnp.sin(ang)
    nr = a1r - 1.0
    ni = a1i
    big = jnp.abs(lre) >= jnp.abs(lim)
    u_ = jnp.where(big, lre, lim)
    v_ = jnp.where(big, lim, lre)
    r_ = v_ / u_
    den = u_ + v_ * r_
    cr_ = jnp.where(big, nr + ni * r_, nr * r_ + ni) / den
    ci_ = jnp.where(big, ni - nr * r_, ni * r_ - nr) / den
    tab_ref[8] = jnp.broadcast_to(2.0 * cr_, (8, D))
    tab_ref[9] = jnp.broadcast_to(2.0 * ci_, (8, D))
    pw = [(a1r, a1i)]
    for _ in range(7):
        pw.append(_cmul(pw[-1][0], pw[-1][1], a1r, a1i))
    row = jax.lax.broadcasted_iota(jnp.int32, (8, D), 0)
    apr_ = jnp.zeros((8, D), F32)
    api_ = jnp.zeros((8, D), F32)
    for j in range(8):
        apr_ = jnp.where(row == j, pw[j][0], apr_)
        api_ = jnp.where(row == j, pw[j][1], api_)
    tab_ref[0] = apr_
    tab_ref[1] = api_
    for n, d in enumerate((1, 2, 4)):
        tab_ref[2 + 2 * n] = jnp.where(row >= d, pw[d - 1][0], 0.0)
        tab_ref[3 + 2 * n] = jnp.where(row >= d, pw[d - 1][1], 0.0)
    carry_ref[...] = jnp.zeros_like(carry_ref)

    wait(_S_BRE, _S_BIM, _S_BX0, _S_CRE, _S_CIM)

    def qv(c):
        def f():
            if c < S // TQ:
                q_proj(c, wq_t)
                v_proj(c, wv_t)
        return f

    prep_group(0, [qv(1), qv(2), qv(3), qv(4)])
    ys_copy(0).start()

    kcol = stats["k"].max(axis=0, keepdims=True)
    kcol2 = jnp.broadcast_to(kcol * kcol, (8, D))
    ind = (jax.lax.broadcasted_iota(jnp.int32, (D, 128), 0) // DH
           == jax.lax.broadcasted_iota(jnp.int32, (D, 128), 1)).astype(F32)
    kn2 = jax.lax.dot_general(kcol2, ind, _NN, preferred_element_type=F32,
                              precision=jax.lax.Precision.HIGHEST)
    bound = jnp.sqrt(jnp.max(stats["q"]) * jnp.max(kn2)) * 1.02 + 1.0
    lv = jnp.log2(jnp.max(stats["v"]))
    ok = jnp.logical_and(bound <= 80.0,
                         jnp.logical_and(lv >= bound - 100.0, lv <= 113.0 - bound))
    safe_ref[0] = ok.astype(jnp.int32)
    wait(_S_BX1, _S_WO)

    def att_fast(g, qb):
        q0 = pl.multiple_of(qb * TQ, TQ)
        steps = [(j, kc) for j in range(HG) for kc in range(NCK)]
        ws = {}
        never = jax.lax.broadcasted_iota(jnp.int32, (NV, 128), 1) < (g - 2 * NG)
        prev = [None]

        def get_w(j):
            if j not in ws:
                qrows = qt_ref[pl.ds(pl.multiple_of(g * 128 + j * DH, DH), DH), pl.ds(q0, TQ)]
                parts = []
                if j > 0:
                    parts.append(jnp.zeros((DH * j, TQ), BF16))
                parts.append(qrows)
                if j < HG - 1:
                    parts.append(jnp.zeros((DH * (HG - 1 - j), TQ), BF16))
                ws[j] = jnp.concatenate(parts, axis=0)
            return ws[j]

        def qk(st):
            j, kc = st
            return _dot(k_ref[g, kc * CK + NV:(kc + 1) * CK, :], get_w(j))

        def vpu_scores(j, kc):
            cols = []
            for tt in range(TQ // 128):
                acc = None
                for d in range(DH):
                    term = kb_ref[j, kc, d] * qf_ref[qb, g * HG + j, d:d + 1, tt * 128:(tt + 1) * 128]
                    if acc is not None:
                        acc = acc + term
                    elif prev[0] is None:
                        acc = term
                    else:
                        acc = jnp.where(never, prev[0], term)
                prev[0] = acc
                cols.append(acc)
            return jnp.concatenate(cols, axis=1)

        svals = {}
        for i in range(DEPTH):
            svals[i] = qk(steps[i])
        l = o = None
        for i, (j, kc) in enumerate(steps):
            if i + DEPTH < len(steps):
                svals[i + DEPTH] = qk(steps[i + DEPTH])
            p = jnp.concatenate([jnp.exp2(vpu_scores(j, kc)), jnp.exp2(svals.pop(i))], axis=0)
            hrow = pl.multiple_of(g * 128 + j * DH, DH)
            ps = p.reshape(CK // 8, 8, TQ).sum(axis=0)
            pv = _dot(vt_ref[pl.ds(hrow, DH), kc * CK:(kc + 1) * CK], p.astype(BF16))
            if kc == 0:
                l, o = ps, pv
            else:
                l, o = l + ps, o + pv
            if kc == NCK - 1:
                ot_ref[qb, j * DH:(j + 1) * DH, :] = o
                lt_ref[qb, j * 8:(j + 1) * 8, :] = l

    def att_safe(g, qb):
        q0 = pl.multiple_of(qb * TQ, TQ)
        ck = 512

        def head(j, c):
            qg = qt_ref[pl.ds(pl.multiple_of(g * 128, 128), 128), pl.ds(q0, TQ)]
            rows = jax.lax.broadcasted_iota(jnp.int32, (128, TQ), 0)
            w = jnp.where((rows // DH) == j, qg, jnp.zeros_like(qg))
            hrow = pl.multiple_of(g * 128 + j * DH, DH)
            m = jnp.full((1, TQ), -jnp.inf, F32)
            l = jnp.zeros((1, TQ), F32)
            o = jnp.zeros((DH, TQ), F32)
            for kc in range(S // ck):
                s = _dot(k_ref[g, kc * ck:(kc + 1) * ck, :], w)
                mn = jnp.maximum(m, s.max(axis=0, keepdims=True))
                alpha = jnp.exp2(m - mn)
                p = jnp.exp2(s - mn)
                l = l * alpha + p.sum(axis=0, keepdims=True)
                o = o * alpha + _dot(vt_ref[pl.ds(hrow, DH), kc * ck:(kc + 1) * ck], p.astype(BF16))
                m = mn
            ot_ref[qb, pl.ds(pl.multiple_of(j * DH, DH), DH), :] = o
            first = jax.lax.broadcasted_iota(jnp.int32, (8, TQ), 0) == 0
            lt_ref[qb, pl.ds(pl.multiple_of(j * 8, 8), 8), :] = jnp.where(first, l, 0.0)
            return c

        jax.lax.fori_loop(0, HG, head, 0)

    def group(g, carry):
        def qblock(qb, c):
            jax.lax.cond(safe_ref[0] == 1, lambda: att_fast(g, qb), lambda: att_safe(g, qb))

            @pl.when(g == NG - 1)
            def _():
                out_proj(g, qb)
                oa_copy(qb).start()

            return c

        jax.lax.fori_loop(0, NQB, qblock, 0)

        @pl.when(g < NG - 1)
        def _():
            prep_group(g + 1, [(lambda qb=qb: out_proj(g, qb)) for qb in range(NQB)])
            ys_copy(g + 1).start()

        return carry

    jax.lax.fori_loop(0, NG, group, 0)

    for g in range(NG):
        ys_copy(g).wait()
    for qb in range(NQB):
        oa_copy(qb).wait()


@jax.jit
def pallas_concat_heads__softmax_full_mha__ssm_conv_s5__prompt_kernel(
    A_x: jax.Array,
    A_wqkv: jax.Array,
    A_wo: jax.Array,
    B_x: jax.Array,
    B_Lambda_re: jax.Array,
    B_Lambda_im: jax.Array,
    B_B_re: jax.Array,
    B_B_im: jax.Array,
    B_C_re: jax.Array,
    B_C_im: jax.Array,
    B_log_dt: jax.Array,
    B_Dskip: jax.Array,
):
    hbm = pl.BlockSpec(memory_space=pl.ANY)
    out = pl.pallas_call(
        _kernel,
        in_specs=[hbm] * 12,
        out_specs=hbm,
        out_shape=jax.ShapeDtypeStruct((S, 2 * D), F32),
        scratch_shapes=[
            pltpu.VMEM((S, D), BF16),
            pltpu.VMEM((3, D, D), BF16),
            pltpu.VMEM((D, D), BF16),
            pltpu.VMEM((S, D), BF16),
            pltpu.VMEM((D, D), BF16),
            pltpu.VMEM((D, D), BF16),
            pltpu.VMEM((D, D), BF16),
            pltpu.VMEM((D, D), BF16),
            pltpu.VMEM((D, S), BF16),
            pltpu.VMEM((NG, S, 128), BF16),
            pltpu.VMEM((D, S), BF16),
            pltpu.VMEM((NQB, 128, TQ), F32),
            pltpu.VMEM((NQB, HG * 8, TQ), F32),
            pltpu.VMEM((10, 8, D), F32),
            pltpu.VMEM((2, 8, D), F32),
            pltpu.VMEM((NQB, H, DH, TQ), F32),
            pltpu.VMEM((NG, NCK * NV, 128), BF16),
            pltpu.VMEM((HG, NCK, DH, NV, 128), F32),
            pltpu.VMEM((S, D), F32),
            pltpu.VMEM((S, D), F32),
            pltpu.VMEM((D,), BF16),
            pltpu.VMEM((D,), BF16),
            pltpu.VMEM((D,), BF16),
            pltpu.VMEM((D,), BF16),
            pltpu.SMEM((1,), jnp.int32),
            pltpu.SemaphoreType.DMA((_N_IN_SEMS,)),
            pltpu.SemaphoreType.DMA((NG,)),
            pltpu.SemaphoreType.DMA((NQB,)),
        ],
        compiler_params=pltpu.CompilerParams(
            vmem_limit_bytes=100 * 1024 * 1024,
        ),
    )(A_x.reshape(S, D), A_wqkv, A_wo, B_x.reshape(S, D), B_Lambda_re, B_Lambda_im,
      B_B_re, B_B_im, B_C_re, B_C_im, B_log_dt, B_Dskip)
    return out.reshape(1, S, 2 * D)
```

```python
import math

import jax
import jax.numpy as jnp
import jax.experimental.pallas as pl
import jax.experimental.pallas.tpu as pltpu

F32 = jnp.float32
BF16 = jnp.bfloat16

S = 2048
D = 512
H = 32
DH = 16
TQ = 512
NQB = S // TQ
HG = 8
NG = H // HG
CK = 128
NV = 16
NCK = S // CK
DEPTH = 2
TS = 128
TB = S // NG
SCAN_CHAINS = 2
LOG2E = math.log2(math.e)
QSCALE = (DH ** -0.5) * LOG2E

_NN = (((1,), (0,)), ((), ()))
_NT = (((1,), (1,)), ((), ()))
_TN = (((0,), (0,)), ((), ()))

(_S_WK, _S_X0, _S_WQ, _S_WV, _S_X1, _S_X2, _S_X3, _S_LRE, _S_LIM, _S_LDT, _S_DSK,
 _S_BRE, _S_BIM, _S_BX0, _S_CRE, _S_CIM, _S_BX1, _S_WO) = range(18)
_N_IN_SEMS = 18


def _dot(a, b, dims=_NN):
    return jax.lax.dot_general(a, b, dims, preferred_element_type=F32)


def _pack_rows(x):
    return pltpu.bitcast(x, jnp.uint32)


def _unpack_rows(x):
    return pltpu.bitcast(x, BF16)


def _cmul(ar, ai, br, bi):
    return ar * br - ai * bi, ar * bi + ai * br


def _kernel(x_hbm, wqkv_hbm, wo_hbm, bx_hbm, lre_hbm, lim_hbm, bre_hbm, bim_hbm,
            cre_hbm, cim_hbm, ldt_hbm, dsk_hbm,
            out_hbm,
            x_ref, w_ref, wo_ref, bx_ref, bre_ref, bim_ref, cre_ref, cim_ref,
            qt_ref, k_ref, vt_ref, ot_ref, lt_ref, tab_ref, carry_ref, qf_ref, kv_ref, kb_ref,
            oacc_ref, ys_ref, lre_ref, lim_ref, ldt_ref, dsk_ref,
            safe_ref, in_sems, ys_sems, oa_sems):

    def cp(src, dst, s):
        return pltpu.make_async_copy(src, dst, in_sems.at[s])

    copies = {
        _S_WK: cp(wqkv_hbm.at[:, D:2 * D], w_ref.at[1], _S_WK),
        _S_X0: cp(x_hbm.at[0:TQ], x_ref.at[0:TQ], _S_X0),
        _S_WQ: cp(wqkv_hbm.at[:, 0:D], w_ref.at[0], _S_WQ),
        _S_WV: cp(wqkv_hbm.at[:, 2 * D:3 * D], w_ref.at[2], _S_WV),
        _S_X1: cp(x_hbm.at[TQ:2 * TQ], x_ref.at[TQ:2 * TQ], _S_X1),
        _S_X2: cp(x_hbm.at[2 * TQ:3 * TQ], x_ref.at[2 * TQ:3 * TQ], _S_X2),
        _S_X3: cp(x_hbm.at[3 * TQ:4 * TQ], x_ref.at[3 * TQ:4 * TQ], _S_X3),
        _S_LRE: cp(lre_hbm, lre_ref, _S_LRE),
        _S_LIM: cp(lim_hbm, lim_ref, _S_LIM),
        _S_LDT: cp(ldt_hbm, ldt_ref, _S_LDT),
        _S_DSK: cp(dsk_hbm, dsk_ref, _S_DSK),
        _S_BRE: cp(bre_hbm, bre_ref, _S_BRE),
        _S_BIM: cp(bim_hbm, bim_ref, _S_BIM),
        _S_BX0: cp(bx_hbm.at[0:TB], bx_ref.at[0:TB], _S_BX0),
        _S_CRE: cp(cre_hbm, cre_ref, _S_CRE),
        _S_CIM: cp(cim_hbm, cim_ref, _S_CIM),
        _S_BX1: cp(bx_hbm.at[TB:S], bx_ref.at[TB:S], _S_BX1),
        _S_WO: cp(wo_hbm, wo_ref, _S_WO),
    }
    for c in copies.values():
        c.start()

    def wait(*ids):
        for s_ in ids:
            copies[s_].wait()

    def ys_copy(g):
        r0 = pl.multiple_of(g * TB, TB)
        return pltpu.make_async_copy(ys_ref.at[pl.ds(r0, TB)],
                                     out_hbm.at[pl.ds(r0, TB), D:2 * D], ys_sems.at[g])

    def oa_copy(tile):
        r0 = pl.multiple_of(tile * 128, 128)
        return pltpu.make_async_copy(oacc_ref.at[pl.ds(r0, 128)],
                                     out_hbm.at[pl.ds(r0, 128), 0:D], oa_sems.at[tile])

    def gen_kb(g, lanes):
        blk = pltpu.bitcast(kv_ref[g], jnp.uint32)
        for c in lanes:
            col = jnp.broadcast_to(blk[:, c:c + 1], blk.shape)
            col = pltpu.bitcast(col, BF16).astype(F32)
            kb_ref[c // DH, :, c % DH] = col.reshape(NCK, NV, 128)

    def ssm_b(u):
        r0 = pl.multiple_of(u * TS, TS)
        xb = bx_ref[pl.ds(r0, TS), :]
        ur = _dot(xb, bre_ref[...], _NT).reshape(TS // 8, 8, D)
        ui = _dot(xb, bim_ref[...], _NT).reshape(TS // 8, 8, D)
        return ur, ui

    def ssm_scan(ur, ui, link):
        nl = D // 128
        ta, tb = tab_ref[0, :, 0:128], tab_ref[1, :, 0:128]
        never = jnp.logical_and(ta < tb, tb < ta)
        cs = [(carry_ref[0, :, lt * 128:(lt + 1) * 128], carry_ref[1, :, lt * 128:(lt + 1) * 128])
              for lt in range(nl)]
        hr = [[None] * nl for _ in range(TS // 8)]
        hi = [[None] * nl for _ in range(TS // 8)]
        for j in range(TS // 8):
            for lt in range(nl):
                sl = slice(lt * 128, (lt + 1) * 128)
                ch = lt * SCAN_CHAINS // nl
                xr = ur[j][:, sl]
                xi = ui[j][:, sl]
                if link[ch] is not None:
                    xr = jnp.where(never, link[ch], xr)
                for n, d in enumerate((1, 2, 4)):
                    mr = tab_ref[2 + 2 * n, :, sl]
                    mi = tab_ref[3 + 2 * n, :, sl]
                    sr = pltpu.roll(xr, d, 0)
                    si = pltpu.roll(xi, d, 0)
                    xr, xi = xr + (mr * sr - mi * si), xi + (mr * si + mi * sr)
                apr = tab_ref[0, :, sl]
                api = tab_ref[1, :, sl]
                cr, ci = cs[lt]
                gr = xr + (apr * cr - api * ci)
                gi = xi + (apr * ci + api * cr)
                c2r = tab_ref[8, :, sl]
                c2i = tab_ref[9, :, sl]
                hr[j][lt] = c2r * gr - c2i * gi
                hi[j][lt] = -(c2r * gi + c2i * gr)
                cs[lt] = (jnp.broadcast_to(gr[7:8, :], (8, 128)), jnp.broadcast_to(gi[7:8, :], (8, 128)))
                link[ch] = gr
        for lt in range(nl):
            carry_ref[0, :, lt * 128:(lt + 1) * 128] = cs[lt][0]
            carry_ref[1, :, lt * 128:(lt + 1) * 128] = cs[lt][1]
        cat = lambda h: jnp.concatenate([jnp.concatenate(r, axis=1) for r in h], axis=0).astype(BF16)
        return cat(hr), cat(hi)

    def ssm_out(u, hr, hi):
        r0 = pl.multiple_of(u * TS, TS)
        xb = bx_ref[pl.ds(r0, TS), :]
        skip = (xb.astype(F32) * dsk_ref[...].astype(F32).reshape(1, D)).astype(BF16).astype(F32)
        ys_ref[pl.ds(r0, TS), :] = (_dot(hr, cre_ref[...], _NT) + _dot(hi, cim_ref[...], _NT) + skip)

    def out_proj(g, qb, t0=0, nt=TQ // 128):
        q0 = pl.multiple_of(qb * TQ + t0 * 128, 128)
        w0 = pl.multiple_of(g * 128, 128)
        cols = slice(t0 * 128, (t0 + nt) * 128)
        rec = 1.0 / lt_ref[qb, :, cols].reshape(HG, 8, nt * 128).sum(axis=1)
        on = jnp.concatenate([ot_ref[qb, j * DH:(j + 1) * DH, cols] * rec[j:j + 1, :] for j in range(HG)],
                             axis=0).astype(BF16)
        contrib = _dot(on, wo_ref[pl.ds(w0, 128), :], _TN)
        old = jnp.where(g == 0, 0.0, oacc_ref[pl.ds(q0, nt * 128), :])
        oacc_ref[pl.ds(q0, nt * 128), :] = old + contrib

    def prep_group(g, extra):
        n = TB // TS
        u0 = g * n
        per = 128 // n
        us = [ssm_b(u0 + u) for u in range(n)]
        for u in range(n):
            extra[u]()
        link = [None] * SCAN_CHAINS
        hs = []
        for u in range(n):
            gen_kb(g, range(u * per, (u + 1) * per))
            hs.append(ssm_scan(*us[u], link))
        for u in range(n):
            ssm_out(u0 + u, *hs[u])

    stats = {"q": jnp.zeros((H, 128), F32), "k": jnp.zeros((8, D), F32), "v": jnp.zeros((8, 128), F32)}

    def k_proj(c):
        kc = _dot(x_ref[c * TQ:(c + 1) * TQ, :], w_ref[1]).astype(BF16)
        for g in range(NG):
            k_ref[g, c * TQ // 2:(c + 1) * TQ // 2, :] = _pack_rows(kc[:, g * 128:(g + 1) * 128])
            for u in range(TQ // CK):
                r0 = (c * (TQ // CK) + u) * NV
                kv_ref[g, r0:r0 + NV, :] = kc[u * CK:u * CK + NV, g * 128:(g + 1) * 128]
        stats["k"] = jnp.maximum(stats["k"], jnp.abs(kc.astype(F32)).reshape(TQ // 8, 8, D).max(axis=0))

    def q_proj(c, wq_t):
        qc = (_dot(wq_t, x_ref[c * TQ:(c + 1) * TQ, :], _NT) * QSCALE).astype(BF16)
        qt_ref[:, c * TQ:(c + 1) * TQ] = _pack_rows(qc)
        qf = qc.astype(F32).reshape(H, DH, TQ)
        qf_ref[c] = qf
        qn = (qf * qf).sum(axis=1)
        for t in range(TQ // 128):
            stats["q"] = jnp.maximum(stats["q"], qn[:, t * 128:(t + 1) * 128])

    def v_proj(c, wv_t):
        vc = _dot(wv_t, x_ref[c * TQ:(c + 1) * TQ, :], _NT).astype(BF16)
        vt_ref[:, c * TQ:(c + 1) * TQ] = _pack_rows(vc)
        va = jnp.abs(vc.astype(F32)).reshape(D // 8, 8, TQ).max(axis=0)
        for t in range(TQ // 128):
            stats["v"] = jnp.maximum(stats["v"], va[:, t * 128:(t + 1) * 128])

    wait(_S_WK, _S_X0)
    k_proj(0)
    wait(_S_WQ, _S_WV)
    wq_t = w_ref[0].T
    wv_t = w_ref[2].T
    q_proj(0, wq_t)
    v_proj(0, wv_t)
    wait(_S_X1, _S_X2, _S_X3, _S_LRE, _S_LIM, _S_LDT, _S_DSK)
    for c in range(1, S // TQ):
        k_proj(c)

    lre = lre_ref[...].astype(F32).reshape(1, D)
    lim = lim_ref[...].astype(F32).reshape(1, D)
    dt = jnp.exp(ldt_ref[...].astype(F32).reshape(1, D)).astype(BF16).astype(F32)
    mag = jnp.exp(dt * lre)
    ang = dt * lim
    a1r = mag * jnp.cos(ang)
    a1i = mag * jnp.sin(ang)
    nr = a1r - 1.0
    ni = a1i
    big = jnp.abs(lre) >= jnp.abs(lim)
    u_ = jnp.where(big, lre, lim)
    v_ = jnp.where(big, lim, lre)
    r_ = v_ / u_
    den = u_ + v_ * r_
    cr_ = jnp.where(big, nr + ni * r_, nr * r_ + ni) / den
    ci_ = jnp.where(big, ni - nr * r_, ni * r_ - nr) / den
    tab_ref[8] = jnp.broadcast_to(2.0 * cr_, (8, D))
    tab_ref[9] = jnp.broadcast_to(2.0 * ci_, (8, D))
    pw = [(a1r, a1i)]
    for _ in range(7):
        pw.append(_cmul(pw[-1][0], pw[-1][1], a1r, a1i))
    row = jax.lax.broadcasted_iota(jnp.int32, (8, D), 0)
    apr_ = jnp.zeros((8, D), F32)
    api_ = jnp.zeros((8, D), F32)
    for j in range(8):
        apr_ = jnp.where(row == j, pw[j][0], apr_)
        api_ = jnp.where(row == j, pw[j][1], api_)
    tab_ref[0] = apr_
    tab_ref[1] = api_
    for n, d in enumerate((1, 2, 4)):
        tab_ref[2 + 2 * n] = jnp.where(row >= d, pw[d - 1][0], 0.0)
        tab_ref[3 + 2 * n] = jnp.where(row >= d, pw[d - 1][1], 0.0)
    carry_ref[...] = jnp.zeros_like(carry_ref)

    wait(_S_BRE, _S_BIM, _S_BX0, _S_CRE, _S_CIM)

    def qv(c):
        def f():
            if c < S // TQ:
                q_proj(c, wq_t)
                v_proj(c, wv_t)
        return f

    prep_group(0, [qv(1), qv(2), qv(3), qv(4)])
    ys_copy(0).start()

    kcol = stats["k"].max(axis=0, keepdims=True)
    kcol2 = jnp.broadcast_to(kcol * kcol, (8, D))
    ind = (jax.lax.broadcasted_iota(jnp.int32, (D, 128), 0) // DH
           == jax.lax.broadcasted_iota(jnp.int32, (D, 128), 1)).astype(F32)
    kn2 = jax.lax.dot_general(kcol2, ind, _NN, preferred_element_type=F32,
                              precision=jax.lax.Precision.HIGHEST)
    bound = jnp.sqrt(jnp.max(stats["q"]) * jnp.max(kn2)) * 1.02 + 1.0
    lv = jnp.log2(jnp.max(stats["v"]))
    ok = jnp.logical_and(bound <= 80.0,
                         jnp.logical_and(lv >= bound - 100.0, lv <= 113.0 - bound))
    safe_ref[0] = ok.astype(jnp.int32)
    wait(_S_BX1, _S_WO)

    def att_fast(g, qb):
        q0 = pl.multiple_of(qb * TQ, TQ)
        steps = [(j, kc) for j in range(HG) for kc in range(NCK)]
        ws = {}
        never = jax.lax.broadcasted_iota(jnp.int32, (NV, 128), 1) < (g - 2 * NG)
        prev = [None]

        def get_w(j):
            if j not in ws:
                qrows = _unpack_rows(qt_ref[pl.ds(pl.multiple_of(g * 64 + j * 8, 8), 8), pl.ds(q0, TQ)])
                parts = []
                if j > 0:
                    parts.append(jnp.zeros((DH * j, TQ), BF16))
                parts.append(qrows)
                if j < HG - 1:
                    parts.append(jnp.zeros((DH * (HG - 1 - j), TQ), BF16))
                ws[j] = jnp.concatenate(parts, axis=0)
            return ws[j]

        def qk(st):
            j, kc = st
            return _dot(_unpack_rows(k_ref[g, (kc * CK + NV) // 2:(kc + 1) * CK // 2, :]), get_w(j))

        def vpu_scores(j, kc):
            cols = []
            for tt in range(TQ // 128):
                acc = None
                tail = None
                for d in range(DH):
                    term = kb_ref[j, kc, d] * qf_ref[qb, g * HG + j, d:d + 1, tt * 128:(tt + 1) * 128]
                    if d == DH - 2:
                        tail = term
                        continue
                    if d == DH - 1:
                        term = tail + term
                    if acc is not None:
                        acc = acc + term
                    elif prev[0] is None:
                        acc = term
                    else:
                        acc = jnp.where(never, prev[0], term)
                prev[0] = acc
                cols.append(acc)
            return jnp.concatenate(cols, axis=1)

        svals = {}
        for i in range(DEPTH):
            svals[i] = qk(steps[i])
        l = o = None
        for i, (j, kc) in enumerate(steps):
            if i + DEPTH < len(steps):
                svals[i + DEPTH] = qk(steps[i + DEPTH])
            p = jnp.concatenate([jnp.exp2(vpu_scores(j, kc)), jnp.exp2(svals.pop(i))], axis=0)
            hrow = pl.multiple_of(g * 64 + j * 8, 8)
            ps = p.reshape(CK // 8, 8, TQ).sum(axis=0)
            pv = _dot(_unpack_rows(vt_ref[pl.ds(hrow, 8), kc * CK:(kc + 1) * CK]), p.astype(BF16))
            if kc == 0:
                l, o = ps, pv
            else:
                l, o = l + ps, o + pv
            if kc == NCK - 1:
                ot_ref[qb, j * DH:(j + 1) * DH, :] = o
                lt_ref[qb, j * 8:(j + 1) * 8, :] = l

    def att_safe(g, qb):
        q0 = pl.multiple_of(qb * TQ, TQ)
        ck = 256

        def head(j, c):
            qg = _unpack_rows(qt_ref[pl.ds(pl.multiple_of(g * 64, 64), 64), pl.ds(q0, TQ)])
            rows = jax.lax.broadcasted_iota(jnp.int32, (128, TQ), 0)
            w = jnp.where((rows // DH) == j, qg, jnp.zeros_like(qg))
            hrow = pl.multiple_of(g * 64 + j * 8, 8)

            def chunk(kc, mlo):
                m, l, o = mlo
                k0 = pl.multiple_of(kc * (ck // 2), ck // 2)
                s = _dot(_unpack_rows(k_ref[g, pl.ds(k0, ck // 2), :]), w)
                mn = jnp.maximum(m, s.max(axis=0, keepdims=True))
                alpha = jnp.exp2(m - mn)
                p = jnp.exp2(s - mn)
                v = _unpack_rows(vt_ref[pl.ds(hrow, 8), pl.ds(pl.multiple_of(kc * ck, ck), ck)])
                return (mn, l * alpha + p.sum(axis=0, keepdims=True), o * alpha + _dot(v, p.astype(BF16)))

            init = (jnp.full((1, TQ), -jnp.inf, F32), jnp.zeros((1, TQ), F32), jnp.zeros((DH, TQ), F32))
            _, l, o = jax.lax.fori_loop(0, S // ck, chunk, init)
            ot_ref[qb, pl.ds(pl.multiple_of(j * DH, DH), DH), :] = o
            first = jax.lax.broadcasted_iota(jnp.int32, (8, TQ), 0) == 0
            lt_ref[qb, pl.ds(pl.multiple_of(j * 8, 8), 8), :] = jnp.where(first, l, 0.0)
            return c

        jax.lax.fori_loop(0, HG, head, 0)

    def group(g, carry):
        def qblock(qb, c):
            jax.lax.cond(safe_ref[0] == 1, lambda: att_fast(g, qb), lambda: att_safe(g, qb))

            @pl.when(jnp.logical_and(g == NG - 1, qb == NQB - 2))
            def _():
                for b in range(NQB - 1):
                    out_proj(g, b)
                    for tt in range(TQ // 128):
                        oa_copy(b * (TQ // 128) + tt).start()

            @pl.when(jnp.logical_and(g == NG - 1, qb == NQB - 1))
            def _():
                for tt in range(TQ // 128):
                    out_proj(g, NQB - 1, tt, 1)
                    oa_copy((NQB - 1) * (TQ // 128) + tt).start()

            return c

        jax.lax.fori_loop(0, NQB, qblock, 0)

        @pl.when(g < NG - 1)
        def _():
            prep_group(g + 1, [(lambda qb=qb: out_proj(g, qb)) for qb in range(NQB)])
            ys_copy(g + 1).start()

        return carry

    jax.lax.fori_loop(0, NG, group, 0)

    for g in range(NG):
        ys_copy(g).wait()
    for tile in range(S // 128):
        oa_copy(tile).wait()


@jax.jit
def pallas_concat_heads__softmax_full_mha__ssm_conv_s5__prompt_kernel(
    A_x: jax.Array,
    A_wqkv: jax.Array,
    A_wo: jax.Array,
    B_x: jax.Array,
    B_Lambda_re: jax.Array,
    B_Lambda_im: jax.Array,
    B_B_re: jax.Array,
    B_B_im: jax.Array,
    B_C_re: jax.Array,
    B_C_im: jax.Array,
    B_log_dt: jax.Array,
    B_Dskip: jax.Array,
):
    hbm = pl.BlockSpec(memory_space=pl.ANY)
    out = pl.pallas_call(
        _kernel,
        in_specs=[hbm] * 12,
        out_specs=hbm,
        out_shape=jax.ShapeDtypeStruct((S, 2 * D), F32),
        scratch_shapes=[
            pltpu.VMEM((S, D), BF16),
            pltpu.VMEM((3, D, D), BF16),
            pltpu.VMEM((D, D), BF16),
            pltpu.VMEM((S, D), BF16),
            pltpu.VMEM((D, D), BF16),
            pltpu.VMEM((D, D), BF16),
            pltpu.VMEM((D, D), BF16),
            pltpu.VMEM((D, D), BF16),
            pltpu.VMEM((D // 2, S), jnp.uint32),
            pltpu.VMEM((NG, S // 2, 128), jnp.uint32),
            pltpu.VMEM((D // 2, S), jnp.uint32),
            pltpu.VMEM((NQB, 128, TQ), F32),
            pltpu.VMEM((NQB, HG * 8, TQ), F32),
            pltpu.VMEM((10, 8, D), F32),
            pltpu.VMEM((2, 8, D), F32),
            pltpu.VMEM((NQB, H, DH, TQ), F32),
            pltpu.VMEM((NG, NCK * NV, 128), BF16),
            pltpu.VMEM((HG, NCK, DH, NV, 128), F32),
            pltpu.VMEM((S, D), F32),
            pltpu.VMEM((S, D), F32),
            pltpu.VMEM((D,), BF16),
            pltpu.VMEM((D,), BF16),
            pltpu.VMEM((D,), BF16),
            pltpu.VMEM((D,), BF16),
            pltpu.SMEM((1,), jnp.int32),
            pltpu.SemaphoreType.DMA((_N_IN_SEMS,)),
            pltpu.SemaphoreType.DMA((NG,)),
            pltpu.SemaphoreType.DMA((S // 128,)),
        ],
        compiler_params=pltpu.CompilerParams(
            vmem_limit_bytes=100 * 1024 * 1024,
        ),
    )(A_x.reshape(S, D), A_wqkv, A_wo, B_x.reshape(S, D), B_Lambda_re, B_Lambda_im,
      B_B_re, B_B_im, B_C_re, B_C_im, B_log_dt, B_Dskip)
    return out.reshape(1, S, 2 * D)
```

```python
import math

import jax
import jax.numpy as jnp
import jax.experimental.pallas as pl
import jax.experimental.pallas.tpu as pltpu

F32 = jnp.float32
BF16 = jnp.bfloat16

S = 2048
D = 512
H = 32
DH = 16
TQ = 512
NQB = S // TQ
HG = 8
NG = H // HG
CK = 128
NV = 16
NCK = S // CK
DEPTH = 2
TS = 128
TB = S // NG
SCAN_CHAINS = 2
LOG2E = math.log2(math.e)
QSCALE = (DH ** -0.5) * LOG2E

_NN = (((1,), (0,)), ((), ()))
_NT = (((1,), (1,)), ((), ()))
_TN = (((0,), (0,)), ((), ()))

(_S_WK, _S_X0, _S_WQ, _S_WV, _S_X1, _S_X2, _S_X3, _S_LRE, _S_LIM, _S_LDT, _S_DSK,
 _S_BRE, _S_BIM, _S_BX0, _S_CRE, _S_CIM, _S_BX1, _S_WO) = range(18)
_N_IN_SEMS = 18


def _dot(a, b, dims=_NN):
    return jax.lax.dot_general(a, b, dims, preferred_element_type=F32)


def _pack_rows(x):
    return pltpu.bitcast(x, jnp.uint32)


def _unpack_rows(x):
    return pltpu.bitcast(x, BF16)


def _cmul(ar, ai, br, bi):
    return ar * br - ai * bi, ar * bi + ai * br


def _kernel(x_hbm, wqkv_hbm, wo_hbm, bx_hbm, lre_hbm, lim_hbm, bre_hbm, bim_hbm,
            cre_hbm, cim_hbm, ldt_hbm, dsk_hbm,
            out_hbm,
            x_ref, w_ref, wo_ref, bx_ref, bre_ref, bim_ref, cre_ref, cim_ref,
            qt_ref, k_ref, vt_ref, ot_ref, lt_ref, tab_ref, carry_ref, qf_ref, kv_ref, kb_ref,
            oacc_ref, ys_ref, lre_ref, lim_ref, ldt_ref, dsk_ref,
            safe_ref, in_sems, ys_sems, oa_sems):

    def cp(src, dst, s):
        return pltpu.make_async_copy(src, dst, in_sems.at[s])

    copies = {
        _S_WK: cp(wqkv_hbm.at[:, D:2 * D], w_ref.at[1], _S_WK),
        _S_X0: cp(x_hbm.at[0:TQ], x_ref.at[0:TQ], _S_X0),
        _S_X1: cp(x_hbm.at[TQ:2 * TQ], x_ref.at[TQ:2 * TQ], _S_X1),
        _S_WQ: cp(wqkv_hbm.at[:, 0:D], w_ref.at[0], _S_WQ),
        _S_WV: cp(wqkv_hbm.at[:, 2 * D:3 * D], w_ref.at[2], _S_WV),
        _S_X2: cp(x_hbm.at[2 * TQ:3 * TQ], x_ref.at[2 * TQ:3 * TQ], _S_X2),
        _S_X3: cp(x_hbm.at[3 * TQ:4 * TQ], x_ref.at[3 * TQ:4 * TQ], _S_X3),
        _S_LRE: cp(lre_hbm, lre_ref, _S_LRE),
        _S_LIM: cp(lim_hbm, lim_ref, _S_LIM),
        _S_LDT: cp(ldt_hbm, ldt_ref, _S_LDT),
        _S_DSK: cp(dsk_hbm, dsk_ref, _S_DSK),
        _S_BRE: cp(bre_hbm, bre_ref, _S_BRE),
        _S_BIM: cp(bim_hbm, bim_ref, _S_BIM),
        _S_BX0: cp(bx_hbm.at[0:TB], bx_ref.at[0:TB], _S_BX0),
        _S_CRE: cp(cre_hbm, cre_ref, _S_CRE),
        _S_CIM: cp(cim_hbm, cim_ref, _S_CIM),
        _S_BX1: cp(bx_hbm.at[TB:S], bx_ref.at[TB:S], _S_BX1),
        _S_WO: cp(wo_hbm, wo_ref, _S_WO),
    }
    for c in copies.values():
        c.start()

    def wait(*ids):
        for s_ in ids:
            copies[s_].wait()

    def ys_copy(g):
        r0 = pl.multiple_of(g * TB, TB)
        return pltpu.make_async_copy(ys_ref.at[pl.ds(r0, TB)],
                                     out_hbm.at[pl.ds(r0, TB), D:2 * D], ys_sems.at[g])

    def oa_copy(tile):
        r0 = pl.multiple_of(tile * 128, 128)
        return pltpu.make_async_copy(oacc_ref.at[pl.ds(r0, 128)],
                                     out_hbm.at[pl.ds(r0, 128), 0:D], oa_sems.at[tile])

    def gen_kb(g, lanes):
        blk = pltpu.bitcast(kv_ref[g], jnp.uint32)
        for c in lanes:
            col = jnp.broadcast_to(blk[:, c:c + 1], blk.shape)
            col = pltpu.bitcast(col, BF16).astype(F32)
            kb_ref[c // DH, :, c % DH] = col.reshape(NCK, NV, 128)

    def ssm_b(u):
        r0 = pl.multiple_of(u * TS, TS)
        xb = bx_ref[pl.ds(r0, TS), :]
        ur = _dot(xb, bre_ref[...], _NT).reshape(TS // 8, 8, D)
        ui = _dot(xb, bim_ref[...], _NT).reshape(TS // 8, 8, D)
        return ur, ui

    def ssm_scan(ur, ui, link):
        nl = D // 128
        ta, tb = tab_ref[0, :, 0:128], tab_ref[1, :, 0:128]
        never = jnp.logical_and(ta < tb, tb < ta)
        cs = [(carry_ref[0, :, lt * 128:(lt + 1) * 128], carry_ref[1, :, lt * 128:(lt + 1) * 128])
              for lt in range(nl)]
        hr = [[None] * nl for _ in range(TS // 8)]
        hi = [[None] * nl for _ in range(TS // 8)]
        for j in range(TS // 8):
            for lt in range(nl):
                sl = slice(lt * 128, (lt + 1) * 128)
                ch = lt * SCAN_CHAINS // nl
                xr = ur[j][:, sl]
                xi = ui[j][:, sl]
                if link[ch] is not None:
                    xr = jnp.where(never, link[ch], xr)
                for n, d in enumerate((1, 2, 4)):
                    mr = tab_ref[2 + 2 * n, :, sl]
                    mi = tab_ref[3 + 2 * n, :, sl]
                    sr = pltpu.roll(xr, d, 0)
                    si = pltpu.roll(xi, d, 0)
                    xr, xi = xr + (mr * sr - mi * si), xi + (mr * si + mi * sr)
                apr = tab_ref[0, :, sl]
                api = tab_ref[1, :, sl]
                cr, ci = cs[lt]
                gr = xr + (apr * cr - api * ci)
                gi = xi + (apr * ci + api * cr)
                c2r = tab_ref[8, :, sl]
                c2i = tab_ref[9, :, sl]
                hr[j][lt] = c2r * gr - c2i * gi
                hi[j][lt] = -(c2r * gi + c2i * gr)
                cs[lt] = (jnp.broadcast_to(gr[7:8, :], (8, 128)), jnp.broadcast_to(gi[7:8, :], (8, 128)))
                link[ch] = gr
        for lt in range(nl):
            carry_ref[0, :, lt * 128:(lt + 1) * 128] = cs[lt][0]
            carry_ref[1, :, lt * 128:(lt + 1) * 128] = cs[lt][1]
        cat = lambda h: jnp.concatenate([jnp.concatenate(r, axis=1) for r in h], axis=0).astype(BF16)
        return cat(hr), cat(hi)

    def ssm_out(u, hr, hi):
        r0 = pl.multiple_of(u * TS, TS)
        xb = bx_ref[pl.ds(r0, TS), :]
        skip = (xb.astype(F32) * dsk_ref[...].astype(F32).reshape(1, D)).astype(BF16).astype(F32)
        ys_ref[pl.ds(r0, TS), :] = (_dot(hr, cre_ref[...], _NT) + _dot(hi, cim_ref[...], _NT) + skip)

    def out_proj(g, qb, t0=0, nt=TQ // 128):
        q0 = pl.multiple_of(qb * TQ + t0 * 128, 128)
        w0 = pl.multiple_of(g * 128, 128)
        cols = slice(t0 * 128, (t0 + nt) * 128)
        rec = 1.0 / lt_ref[qb, :, cols].reshape(HG, 8, nt * 128).sum(axis=1)
        on = jnp.concatenate([ot_ref[qb, j * DH:(j + 1) * DH, cols] * rec[j:j + 1, :] for j in range(HG)],
                             axis=0).astype(BF16)
        contrib = _dot(on, wo_ref[pl.ds(w0, 128), :], _TN)
        old = jnp.where(g == 0, 0.0, oacc_ref[pl.ds(q0, nt * 128), :])
        oacc_ref[pl.ds(q0, nt * 128), :] = old + contrib

    def prep_group(g, extra):
        n = TB // TS
        u0 = g * n
        per = 128 // n
        us = [ssm_b(u0 + u) for u in range(n)]
        for u in range(n):
            extra[u]()
        link = [None] * SCAN_CHAINS
        hs = []
        for u in range(n):
            gen_kb(g, range(u * per, (u + 1) * per))
            hs.append(ssm_scan(*us[u], link))
        for u in range(n):
            ssm_out(u0 + u, *hs[u])

    stats = {"q": jnp.zeros((H, 128), F32), "k": jnp.zeros((8, D), F32), "v": jnp.zeros((8, 128), F32)}

    def k_proj(c):
        kc = _dot(x_ref[c * TQ:(c + 1) * TQ, :], w_ref[1]).astype(BF16)
        for g in range(NG):
            k_ref[g, c * TQ // 2:(c + 1) * TQ // 2, :] = _pack_rows(kc[:, g * 128:(g + 1) * 128])
            for u in range(TQ // CK):
                r0 = (c * (TQ // CK) + u) * NV
                kv_ref[g, r0:r0 + NV, :] = kc[u * CK:u * CK + NV, g * 128:(g + 1) * 128]
        stats["k"] = jnp.maximum(stats["k"], jnp.abs(kc.astype(F32)).reshape(TQ // 8, 8, D).max(axis=0))

    def q_proj(c, wq_t):
        qc = (_dot(wq_t, x_ref[c * TQ:(c + 1) * TQ, :], _NT) * QSCALE).astype(BF16)
        qt_ref[:, c * TQ:(c + 1) * TQ] = _pack_rows(qc)
        qf = qc.astype(F32).reshape(H, DH, TQ)
        qf_ref[c] = qf
        qn = (qf * qf).sum(axis=1)
        for t in range(TQ // 128):
            stats["q"] = jnp.maximum(stats["q"], qn[:, t * 128:(t + 1) * 128])

    def v_proj(c, wv_t):
        vc = _dot(wv_t, x_ref[c * TQ:(c + 1) * TQ, :], _NT).astype(BF16)
        vt_ref[:, c * TQ:(c + 1) * TQ] = _pack_rows(vc)
        va = jnp.abs(vc.astype(F32)).reshape(D // 8, 8, TQ).max(axis=0)
        for t in range(TQ // 128):
            stats["v"] = jnp.maximum(stats["v"], va[:, t * 128:(t + 1) * 128])

    wait(_S_WK, _S_X0)
    k_proj(0)
    wait(_S_X1, _S_WQ)
    k_proj(1)
    wq_t = w_ref[0].T
    q_proj(0, wq_t)
    q_proj(1, wq_t)
    wait(_S_WV, _S_X2, _S_X3, _S_LRE, _S_LIM, _S_LDT, _S_DSK)
    k_proj(2)
    k_proj(3)
    wv_t = w_ref[2].T
    v_proj(0, wv_t)
    v_proj(1, wv_t)

    kcol = stats["k"].max(axis=0, keepdims=True)
    kcol2 = jnp.broadcast_to(kcol * kcol, (8, D))
    ind = (jax.lax.broadcasted_iota(jnp.int32, (D, 128), 0) // DH
           == jax.lax.broadcasted_iota(jnp.int32, (D, 128), 1)).astype(F32)
    kn2 = jax.lax.dot_general(kcol2, ind, _NN, preferred_element_type=F32,
                              precision=jax.lax.Precision.HIGHEST)
    kn2max = jnp.max(kn2, axis=1, keepdims=True)[0:1, :]

    lre = lre_ref[...].astype(F32).reshape(1, D)
    lim = lim_ref[...].astype(F32).reshape(1, D)
    dt = jnp.exp(ldt_ref[...].astype(F32).reshape(1, D)).astype(BF16).astype(F32)
    mag = jnp.exp(dt * lre)
    ang = dt * lim
    a1r = mag * jnp.cos(ang)
    a1i = mag * jnp.sin(ang)
    nr = a1r - 1.0
    ni = a1i
    big = jnp.abs(lre) >= jnp.abs(lim)
    u_ = jnp.where(big, lre, lim)
    v_ = jnp.where(big, lim, lre)
    r_ = v_ / u_
    den = u_ + v_ * r_
    cr_ = jnp.where(big, nr + ni * r_, nr * r_ + ni) / den
    ci_ = jnp.where(big, ni - nr * r_, ni * r_ - nr) / den
    tab_ref[8] = jnp.broadcast_to(2.0 * cr_, (8, D))
    tab_ref[9] = jnp.broadcast_to(2.0 * ci_, (8, D))
    pw = [(a1r, a1i)]
    for _ in range(7):
        pw.append(_cmul(pw[-1][0], pw[-1][1], a1r, a1i))
    row = jax.lax.broadcasted_iota(jnp.int32, (8, D), 0)
    apr_ = jnp.zeros((8, D), F32)
    api_ = jnp.zeros((8, D), F32)
    for j in range(8):
        apr_ = jnp.where(row == j, pw[j][0], apr_)
        api_ = jnp.where(row == j, pw[j][1], api_)
    tab_ref[0] = apr_
    tab_ref[1] = api_
    for n, d in enumerate((1, 2, 4)):
        tab_ref[2 + 2 * n] = jnp.where(row >= d, pw[d - 1][0], 0.0)
        tab_ref[3 + 2 * n] = jnp.where(row >= d, pw[d - 1][1], 0.0)
    carry_ref[...] = jnp.zeros_like(carry_ref)

    wait(_S_BRE, _S_BIM, _S_BX0, _S_CRE, _S_CIM)

    def qv(c):
        def f():
            q_proj(c, wq_t)
            v_proj(c, wv_t)
        return f

    prep_group(0, [qv(2), qv(3), lambda: None, lambda: None])
    ys_copy(0).start()

    qmax = jnp.max(jnp.max(stats["q"], axis=0, keepdims=True), axis=1, keepdims=True)
    vmax = jnp.max(jnp.max(stats["v"], axis=0, keepdims=True), axis=1, keepdims=True)
    bound = jnp.sqrt(qmax * kn2max) * 1.02 + 1.0
    lv = jnp.log2(vmax)
    ok = jnp.logical_and(bound <= 80.0,
                         jnp.logical_and(lv >= bound - 100.0, lv <= 113.0 - bound))
    safe_ref[0] = jnp.max(ok.astype(jnp.int32))
    wait(_S_BX1, _S_WO)

    def att_fast(g, qb):
        q0 = pl.multiple_of(qb * TQ, TQ)
        steps = [(j, kc) for j in range(HG) for kc in range(NCK)]
        ws = {}
        never = jax.lax.broadcasted_iota(jnp.int32, (NV, 128), 1) < (g - 2 * NG)
        prev = [None]

        def get_w(j):
            if j not in ws:
                qrows = _unpack_rows(qt_ref[pl.ds(pl.multiple_of(g * 64 + j * 8, 8), 8), pl.ds(q0, TQ)])
                parts = []
                if j > 0:
                    parts.append(jnp.zeros((DH * j, TQ), BF16))
                parts.append(qrows)
                if j < HG - 1:
                    parts.append(jnp.zeros((DH * (HG - 1 - j), TQ), BF16))
                ws[j] = jnp.concatenate(parts, axis=0)
            return ws[j]

        def qk(st):
            j, kc = st
            return _dot(_unpack_rows(k_ref[g, (kc * CK + NV) // 2:(kc + 1) * CK // 2, :]), get_w(j))

        def vpu_scores(j, kc):
            cols = []
            for tt in range(TQ // 128):
                acc = None
                tail = None
                for d in range(DH):
                    term = kb_ref[j, kc, d] * qf_ref[qb, g * HG + j, d:d + 1, tt * 128:(tt + 1) * 128]
                    if d == DH - 2:
                        tail = term
                        continue
                    if d == DH - 1:
                        term = tail + term
                    if acc is not None:
                        acc = acc + term
                    elif prev[0] is None:
                        acc = term
                    else:
                        acc = jnp.where(never, prev[0], term)
                prev[0] = acc
                cols.append(acc)
            return jnp.concatenate(cols, axis=1)

        svals = {}
        for i in range(DEPTH):
            svals[i] = qk(steps[i])
        l = o = None
        for i, (j, kc) in enumerate(steps):
            if i + DEPTH < len(steps):
                svals[i + DEPTH] = qk(steps[i + DEPTH])
            p = jnp.concatenate([jnp.exp2(vpu_scores(j, kc)), jnp.exp2(svals.pop(i))], axis=0)
            hrow = pl.multiple_of(g * 64 + j * 8, 8)
            ps = p.reshape(CK // 8, 8, TQ).sum(axis=0)
            pv = _dot(_unpack_rows(vt_ref[pl.ds(hrow, 8), kc * CK:(kc + 1) * CK]), p.astype(BF16))
            if kc == 0:
                l, o = ps, pv
            else:
                l, o = l + ps, o + pv
            if kc == NCK - 1:
                ot_ref[qb, j * DH:(j + 1) * DH, :] = o
                lt_ref[qb, j * 8:(j + 1) * 8, :] = l

    def att_safe(g, qb):
        q0 = pl.multiple_of(qb * TQ, TQ)
        ck = 256

        def head(j, c):
            qg = _unpack_rows(qt_ref[pl.ds(pl.multiple_of(g * 64, 64), 64), pl.ds(q0, TQ)])
            rows = jax.lax.broadcasted_iota(jnp.int32, (128, TQ), 0)
            w = jnp.where((rows // DH) == j, qg, jnp.zeros_like(qg))
            hrow = pl.multiple_of(g * 64 + j * 8, 8)

            def chunk(kc, mlo):
                m, l, o = mlo
                k0 = pl.multiple_of(kc * (ck // 2), ck // 2)
                s = _dot(_unpack_rows(k_ref[g, pl.ds(k0, ck // 2), :]), w)
                mn = jnp.maximum(m, s.max(axis=0, keepdims=True))
                alpha = jnp.exp2(m - mn)
                p = jnp.exp2(s - mn)
                v = _unpack_rows(vt_ref[pl.ds(hrow, 8), pl.ds(pl.multiple_of(kc * ck, ck), ck)])
                return (mn, l * alpha + p.sum(axis=0, keepdims=True), o * alpha + _dot(v, p.astype(BF16)))

            init = (jnp.full((1, TQ), -jnp.inf, F32), jnp.zeros((1, TQ), F32), jnp.zeros((DH, TQ), F32))
            _, l, o = jax.lax.fori_loop(0, S // ck, chunk, init)
            ot_ref[qb, pl.ds(pl.multiple_of(j * DH, DH), DH), :] = o
            first = jax.lax.broadcasted_iota(jnp.int32, (8, TQ), 0) == 0
            lt_ref[qb, pl.ds(pl.multiple_of(j * 8, 8), 8), :] = jnp.where(first, l, 0.0)
            return c

        jax.lax.fori_loop(0, HG, head, 0)

    def group(g, carry):
        def qblock(qb, c):
            jax.lax.cond(safe_ref[0] == 1, lambda: att_fast(g, qb), lambda: att_safe(g, qb))

            @pl.when(jnp.logical_and(g == NG - 1, qb == NQB - 2))
            def _():
                for b in range(NQB - 1):
                    out_proj(g, b)
                    for tt in range(TQ // 128):
                        oa_copy(b * (TQ // 128) + tt).start()

            @pl.when(jnp.logical_and(g == NG - 1, qb == NQB - 1))
            def _():
                for tt in range(TQ // 128):
                    out_proj(g, NQB - 1, tt, 1)
                    oa_copy((NQB - 1) * (TQ // 128) + tt).start()

            return c

        jax.lax.fori_loop(0, NQB, qblock, 0)

        @pl.when(g < NG - 1)
        def _():
            prep_group(g + 1, [(lambda qb=qb: out_proj(g, qb)) for qb in range(NQB)])
            ys_copy(g + 1).start()

        return carry

    jax.lax.fori_loop(0, NG, group, 0)

    for g in range(NG):
        ys_copy(g).wait()
    for tile in range(S // 128):
        oa_copy(tile).wait()


@jax.jit
def pallas_concat_heads__softmax_full_mha__ssm_conv_s5__prompt_kernel(
    A_x: jax.Array,
    A_wqkv: jax.Array,
    A_wo: jax.Array,
    B_x: jax.Array,
    B_Lambda_re: jax.Array,
    B_Lambda_im: jax.Array,
    B_B_re: jax.Array,
    B_B_im: jax.Array,
    B_C_re: jax.Array,
    B_C_im: jax.Array,
    B_log_dt: jax.Array,
    B_Dskip: jax.Array,
):
    hbm = pl.BlockSpec(memory_space=pl.ANY)
    out = pl.pallas_call(
        _kernel,
        in_specs=[hbm] * 12,
        out_specs=hbm,
        out_shape=jax.ShapeDtypeStruct((S, 2 * D), F32),
        scratch_shapes=[
            pltpu.VMEM((S, D), BF16),
            pltpu.VMEM((3, D, D), BF16),
            pltpu.VMEM((D, D), BF16),
            pltpu.VMEM((S, D), BF16),
            pltpu.VMEM((D, D), BF16),
            pltpu.VMEM((D, D), BF16),
            pltpu.VMEM((D, D), BF16),
            pltpu.VMEM((D, D), BF16),
            pltpu.VMEM((D // 2, S), jnp.uint32),
            pltpu.VMEM((NG, S // 2, 128), jnp.uint32),
            pltpu.VMEM((D // 2, S), jnp.uint32),
            pltpu.VMEM((NQB, 128, TQ), F32),
            pltpu.VMEM((NQB, HG * 8, TQ), F32),
            pltpu.VMEM((10, 8, D), F32),
            pltpu.VMEM((2, 8, D), F32),
            pltpu.VMEM((NQB, H, DH, TQ), F32),
            pltpu.VMEM((NG, NCK * NV, 128), BF16),
            pltpu.VMEM((HG, NCK, DH, NV, 128), F32),
            pltpu.VMEM((S, D), F32),
            pltpu.VMEM((S, D), F32),
            pltpu.VMEM((D,), BF16),
            pltpu.VMEM((D,), BF16),
            pltpu.VMEM((D,), BF16),
            pltpu.VMEM((D,), BF16),
            pltpu.SMEM((1,), jnp.int32),
            pltpu.SemaphoreType.DMA((_N_IN_SEMS,)),
            pltpu.SemaphoreType.DMA((NG,)),
            pltpu.SemaphoreType.DMA((S // 128,)),
        ],
        compiler_params=pltpu.CompilerParams(
            vmem_limit_bytes=100 * 1024 * 1024,
        ),
    )(A_x.reshape(S, D), A_wqkv, A_wo, B_x.reshape(S, D), B_Lambda_re, B_Lambda_im,
      B_B_re, B_B_im, B_C_re, B_C_im, B_log_dt, B_Dskip)
    return out.reshape(1, S, 2 * D)
```
